```python
import os as _os
_os.environ.setdefault('JAX_PLATFORMS', 'cpu')
import jax
import jax.numpy as jnp

def _softmax(x, axis=-1):
    return jax.nn.softmax(x, axis=axis)

def _gelu(x):
    return jax.nn.gelu(x, approximate=True)

def _silu(x):
    return jax.nn.silu(x)

def _sigmoid(x):
    return jax.nn.sigmoid(x)

def _layernorm(x, axis=-1, eps=1e-05):
    m = jnp.mean(x, axis=axis, keepdims=True)
    v = jnp.var(x, axis=axis, keepdims=True)
    return (x - m) / jnp.sqrt(v + eps)

def _scatter_add(tgt, idx, src, axis=0):
    return tgt.at[idx].add(src)

def _segment_sum(src, seg, n):
    return jax.ops.segment_sum(src, seg, n)

class _Rng:

    def __init__(self, key):
        self._k = key

    def _next(self):
        self._k, sub = jax.random.split(self._k)
        return sub

    def normal(self, shape):
        return jax.random.normal(self._next(), shape, dtype=jnp.bfloat16)

    def randint(self, lo, hi, shape):
        return jax.random.randint(self._next(), shape, lo, hi, dtype=jnp.int32)

    def uniform(self, shape, lo=0.0, hi=1.0):
        return jax.random.uniform(self._next(), shape, jnp.bfloat16, lo, hi)

    def permutation(self, n):
        return jax.random.permutation(self._next(), n)
kernel_name = 'standalone__window_attn_twins__vision'

def setup_inputs():
    _rng = _Rng(jax.random.key(int.from_bytes(__import__("os").urandom(4), "little")))
    _w = lambda a: (lambda t: t.astype(jnp.bfloat16) if jnp.issubdtype(t.dtype, jnp.floating) else t)(jnp.asarray(a))
    H = W = 384 // 8 * 8
    C = 96
    return {'x': _w((lambda *s: _rng.normal(s) * 0.4)(1, H, W, C)), 'wq': _w((lambda *s: _rng.normal(s) * 0.4)(C, C)), 'wkv': _w((lambda *s: _rng.normal(s) * 0.4)(C, 2 * C)), 'wo': _w((lambda *s: _rng.normal(s) * 0.05)(C, C))}

def reference(x, wq, wkv, wo):
    B, H, W, C = x.shape
    win = 8
    nh, nw = (H // win, W // win)
    xs = x.reshape(B, nh, win, nw, win, C).mean(axis=(2, 4)).reshape(B, nh * nw, C)
    q = x.reshape(B, H * W, C) @ wq
    kv = xs @ wkv
    k, v = (kv[..., :C].copy(), kv[..., C:].copy())
    scale = C ** (-0.5)
    p = _softmax(jnp.einsum('bqc,bkc->bqk', q, k) * scale, axis=-1)
    o = jnp.einsum('bqk,bkc->bqc', p, v) @ wo
    return o.reshape(B, H, W, C)
```

```python
import functools
import itertools

import jax
import jax.numpy as jnp
import numpy as np
import jax.experimental.pallas as pl
import jax.experimental.pallas.tpu as pltpu

F32, BF16, I32 = jnp.float32, jnp.bfloat16, jnp.int32
WIN = 8
T = 128
SLAB = 16
LOG2E = 1.4426950408889634
LOWEST = float(np.finfo(np.float32).min)

NA = 60
UNROLL = 4
MXUS = 4
MXU_LAT = 131

NM, NK, NT = 2, 6, 6
_SCHEME = """
+10                     | +00 +25 +40 -02 -05 -10     | +00 +10
+00 -10                 | +00 +52 -01 -04 -20 -50     | +00
+01                     | +11 +15 +30 -01 -12 -31     | +01 +11
+01 -11                 | +03 +10 +21 -11 -13 -51     | +11
+02                     | +22 +24 -02 -14 -21 -32     | +02
+12                     | +22 +42 -12 -20 -23 -41     | +12
+13                     | +03 +33 -13 -30 -32 -35 -43 | +03 +13
+03 -13                 | +31 +33 -03 -23 -30 -34 -53 | +03
+04                     | +04 +42 +44 -14 -34 -41 -45 | +04 +14
+04 -14                 | +14 +40 +41 +43 -24 -44 -54 | +14
+05                     | +25 +51 +55 -05 -35 -52 -54 | +05
+15                     | +15 +45 +52 +55 -25 -50 -53 | +15
+01 +10                 | +10 -01                     | +00 -11
+00 +01                 | +01 -30                     | +00 +01
+10 +11                 | +10 -03                     | +10 +11
+00 +02 -10             | +20 -02                     | +00 +10 +12
+00 +02                 | +02 -25                     | +00 +02 +10 +12
+00 +02 -10 -12         | +52 -20                     | +10 +12
+04 -10                 | +04 +40                     | +00 -14
+00 -04                 | +04                         | +00 +04
+14 -10                 | +40                         | +10 +14
+00 +05 -10             | +25 +50 -05 -52             | +00 +10 +15
+00 +05                 | +05 -25                     | +00 +05 +10 +15
+00 +05 -10 -15         | +52 -50                     | +10 +15
+01 -11 -12             | +12 -21                     | +01 +02 +11
+11 +12                 | +12 -41                     | +01 +02 +11 +12
+01 +02 -11 -12         | +21 -14                     | +01 +02
+01 +13                 | +13 +31 -03 -30             | +03 +11
+11 +13                 | +03 -13                     | +11 -13
+01 +03                 | +31 -30                     | +01 -03
+01 +15 -11             | +51 -15                     | +01 +11 -05
+15 -11                 | +15                         | +01 +11 -05 -15
+05 +11 -01 -15         | +51                         | +01 -05
+02 +03 -13             | +23 -32                     | +03 +12 +13
+12 +13 -02 -03         | +23                         | +12 +13
+02 +03                 | +32                         | +02 +03 +12 +13
+04 +12 -14             | +14 +42 -24 -41             | +02 -04 -14
+02 +14 -04 -12         | +14 -24                     | +02 -04
+12 -14                 | +41 -42                     | +02 +12 -04 -14
+04 +13                 | +43 -34                     | +03 -14
+03 +04                 | +34                         | +03 +04
+13 +14                 | +43                         | +13 +14
+03 +05 -13             | +53 -35                     | +03 +13 +15
+03 +05                 | +35                         | +03 +05 +13 +15
+13 +15 -03 -05         | +53                         | +13 +15
+04 +15 -14             | +45 +54                     | +04 +05 +14
+14 -15                 | +45                         | +04 +05 +14 +15
+05 +14 -04 -15         | +54                         | +04 +05
+00 +01 +03 -13         | +03 -30                     | +03 +10 +11 +13
+10 +11 +13 -00 -01 -03 | +03                         | +10 +11 +13
+00 +01 +03             | +30                         | +00 +01 +03 +10 +11 +13
+04 +11 +12             | +41 -14                     | +01 +02 -14
+01 +02 +04             | +14                         | +01 +02 +04
+11 +12 +14             | +41                         | +11 +12 +14
+00 +02 -10 -12 -15     | +25 -52                     | +00 +02 +05 +10 +12
+10 +12 +15             | +25                         | +00 +02 +05 +10 +12 +15
+00 +02 +05 -10 -12 -15 | +52                         | +00 +02 +05
"""
_ORDER = "50 25 52 02 20 05 00 10 40 54 44 04 55 01 45 30 51 15 11 35 53 03 13 31 23 32 12 43 33 34 14 21 41 22 24 42"
GW = 3


def _parse_scheme():
    lines = [line.split("|") for line in _SCHEME.strip().splitlines()]
    mats = [np.zeros((len(lines),) + shape, np.int64) for shape in ((NM, NK), (NK, NT), (NM, NT))]
    for r, fields in enumerate(lines):
        for mat, field in zip(mats, fields):
            for term in field.split():
                mat[r, int(term[1]), int(term[2])] = int(term[0] + "1")
    want = np.einsum("ia,kb,tc->ikbtac", np.eye(NM), np.eye(NK), np.eye(NT))
    assert np.array_equal(np.einsum("rik,rbt,rac->ikbtac", *mats), want)
    return mats


def _plan():
    su, sv, sw = _parse_scheme()
    order = [(int(e[0]), int(e[1])) for e in _ORDER.split()]
    groups = [order[i:i + GW] for i in range(0, len(order), GW)]
    when = {e: s for s, group in enumerate(groups) for e in group}
    terms = [{(int(k), int(t)): int(v[k, t]) for k, t in np.argwhere(v)} for v in sv]
    sums = [{(k, t): 1 for k in range(NK)} for t in range(NT)]
    temps = []
    while True:
        count = {}
        for form in terms + sums:
            for a, b in itertools.combinations(sorted(form), 2):
                key = (a, b, form[a] * form[b])
                count[key] = count.get(key, 0) + 1
        a, b, sign = max(count, key=lambda k: (count[k], -abs(when[k[0]] - when[k[1]])))
        if count[a, b, sign] < 2:
            break
        new = (-1, len(temps))
        when[new] = max(when[a], when[b])
        temps.append((new, a, b, sign))
        for form in terms + sums:
            if a in form and b in form and form[a] * form[b] == sign:
                form[new] = form.pop(a)
                del form[b]
    perm = sorted(range(len(terms)), key=lambda r: (max(when[e] for e in terms[r]), len(terms[r])))
    su, sw, prog = su[perm], sw[perm], []
    for r, form in enumerate(terms[p] for p in perm):
        seq = sorted(form, key=lambda e: (when[e], -form[e]))
        lead = form[seq[0]]
        su[r] *= lead
        prog.append([(when[e], e, form[e] * lead) for e in seq])
    return su, sw, groups, when, temps, prog, [sorted(form, key=when.get) for form in sums]


SU, SW, GROUPS, WHEN, TEMPS, PROG, SUMS = _plan()
R = len(SU)
NS = len(GROUPS)


def _lincomb(coef, value):
    acc = None
    for idx in [tuple(int(a) for a in i) for i in np.concatenate([np.argwhere(coef > 0), np.argwhere(coef < 0)])]:
        v = value(*idx)
        if acc is None:
            acc = v if coef[idx] > 0 else -v
        else:
            acc = acc + v if coef[idx] > 0 else acc - v
    return acc


def _max_over_vregs(a):
    return jnp.max(a.reshape(a.shape[0] // 8, 8, a.shape[1]), axis=0)


def _layout(C, NKT):
    NG, CH = NKT // NK, C // NM
    sizes = dict(S=-(-NG * NS // (R // GW)) * T,
                 B=NG * T // 2,
                 M=CH,
                 A=CH // 2,
                 K=T,
                 L=NG * 64,
                 X=16, H=8, F=16, INV=8, MAX=8, RHO=8, OUT=8, PACE=8, END=0)
    return dict(zip(sizes, (int(r) for r in np.cumsum([0] + list(sizes.values())))))


def _kernel(x_hbm, wq_hbm, wkv_hbm, wo_hbm, o_hbm,
            x_s, o_s, xa_s, wq_s, wkv_s, wo_s, w_s, k_s, v_s, vf_s, a_s, vm_s,
            ring0, ring1, ring2, ring3, buf0, buf1, in_sems, w_sems, out_sem):
    H, C, W = x_hbm.shape
    NTILE = H * W // T
    NKT = k_s.shape[0]
    NG = NKT // NK
    CH = C // NM
    RC = WIN * WIN
    at = _layout(C, NKT)
    bufs = (buf0, buf1)
    bufs16 = tuple(b.bitcast(BF16) for b in bufs)
    a16 = a_s.bitcast(BF16)

    def put(u, r0, c, v):
        u[r0:r0 + v.shape[0], c * T:c * T + v.shape[1]] = pltpu.bitcast(v, I32)

    def get(u, r0, n, c, w=1):
        return pltpu.bitcast(u[r0:r0 + n, c * T:(c + w) * T], F32)

    def put16(u16, r0, c, v):
        u16[r0:r0 + v.shape[0], c * T:c * T + v.shape[1]] = v

    def twice(v):
        return jnp.concatenate([v, v], axis=0)

    def hbm_tiles(ref, n0, n):
        return ref.at[pl.ds(n0 % H, n), :, pl.ds(pl.multiple_of(n0 // H * T, T), T)]

    def in_copy(i):
        return pltpu.make_async_copy(hbm_tiles(x_hbm, i * RC, RC), x_s.at[pl.ds(i * RC, RC)], in_sems.at[i])

    def out_copy(n0, n):
        return pltpu.make_async_copy(o_s.at[pl.ds(n0, n)], hbm_tiles(o_hbm, n0, n), out_sem)

    def splice(load, n, pre):
        out, w0 = [], 0
        for w in sorted(pre) + [n]:
            if w > w0:
                out.append(load(w0, w))
            if w < n:
                out.append(pre[w])
            w0 = w + 1
        return out[0] if len(out) == 1 else jnp.concatenate(out, axis=0)

    def emit(mats, vecs, zero):
        clock, start, pops = [0] * MXUS, [], []
        for n, (rows, _, _) in enumerate(mats):
            unit = int(np.argmin(clock))
            start.append(clock[unit])
            pops += [(clock[unit] + MXU_LAT + o, n, o) for o in range(0, rows, 8)]
            clock[unit] += rows
        pops = np.array(pops)
        todo, last = {}, -1
        for j, (cycle, after, before, *_) in enumerate(vecs):
            src = None
            last = max(last, after)
            if cycle >= MXU_LAT:
                ok = pops[pops[:, 1] < before]
                src = tuple(int(e) for e in ok[np.argmin(np.abs(ok[:, 0] - cycle)), 1:])
                last = max(last, src[0])
            assert last < before
            todo.setdefault(last, []).append((j, src))
        vals, pre, rows_at = [], {}, {}
        for n in range(-1, len(mats)):
            if n >= 0:
                vals.append(mats[n][1](pre.pop(n, {})))
            for j, src in todo.get(n, []):
                cycle, _, _, u, par, row, run = vecs[j]
                v = None
                if src is not None:
                    v = vals[src[0]][src[1]:src[1] + 8]
                    if row not in rows_at:
                        rows_at[row] = pl.ds(pl.multiple_of(zero + row, 8), 8)
                    u[rows_at[row], j % 4 * T:(j % 4 + 1) * T] = pltpu.bitcast(v, I32)
                    later = [(start[m] + SLAB * w, m, w) for m in range(n + 1, min(n + 40, len(mats)))
                             for w in range(mats[m][0] // SLAB)
                             if mats[m][2] is not None and w not in pre.get(m, {})
                             and start[m] + SLAB * w >= cycle + 36]
                    if later:
                        _, m, w = min(later)
                        pre.setdefault(m, {})[w] = mats[m][2](par, w)
                run(v)

    w_copies = [pltpu.make_async_copy(src, dst, w_sems.at[i])
                for i, (src, dst) in enumerate(((wq_hbm, wq_s), (wkv_hbm, wkv_s), (wo_hbm, wo_s)))]
    in_copy(0).start()
    for cp in w_copies:
        cp.start()

    AW = R // 4 * 4
    VF0 = -(-NA // AW) * (C + 16)
    assert VF0 + 2 * C <= at["M"]

    def state_pos(n):
        return n // AW * (C + 16), n % AW

    for n in range(0, NA, 4):
        put(buf1, *state_pos(n),
            jnp.concatenate([jnp.zeros((C + 8, 4 * T), F32), jnp.full((8, 4 * T), LOWEST, F32)], axis=0))
    put(buf1, at["M"], 0, jnp.zeros((CH, R * T), F32))
    put(buf1, at["INV"], 0, jnp.zeros((8, NT * T), F32))
    for cp in w_copies:
        cp.wait()
    in_copy(1).start()
    w_s[:C] = (jax.lax.dot_general(wq_s[...], wkv_s[:, :C], (((1,), (1,)), ((), ())),
                                   preferred_element_type=F32) * (C ** -0.5 * LOG2E)).astype(BF16)
    w_s[C:] = jnp.dot(wkv_s[:, C:], wo_s[...], preferred_element_type=F32).T.astype(BF16)

    def pool_ops(i):
        lane = jax.lax.broadcasted_iota(I32, (SLAB, T), 1)
        low = [(lane & (1 << d)) == 0 for d in range(3)]
        level = [[], [], [], []]

        def piece(c, w):
            acc = jnp.sum(x_s[pl.ds(i * RC + w * WIN, WIN), c:c + SLAB, :].astype(F32), axis=0)
            level[0].append(acc)
            for d in range(3):
                if len(level[d]) == 2:
                    a, b = level[d]
                    level[d].clear()
                    level[d + 1].append(jnp.where(low[d], a + pltpu.roll(a, T - (1 << d), 1),
                                                  b + pltpu.roll(b, 1 << d, 1)))
            return acc, ((c, (level[3].pop() * (1.0 / RC)).astype(BF16)) if level[3] else None)
        return [functools.partial(piece, c, w) for c in range(0, C, SLAB) for w in range(WIN)]

    def project_ops(i):
        parts = []

        def part(j, pre):
            parts.append(jnp.dot(w_s[j * CH:(j + 1) * CH], x_s[NTILE], preferred_element_type=F32))
            if j == MXUS - 1:
                kt = jnp.concatenate(parts[:2] + [jnp.zeros((T - C, T), F32)], axis=0)
                vt = jnp.concatenate(parts[2:], axis=0)
                k_s[i] = pltpu.bitcast(kt.T.astype(BF16), I32)
                v_s[...] = pltpu.bitcast(vt.astype(BF16), I32)
                vf_s[...] = vt
            return parts[j]
        return [(CH, functools.partial(part, j), None) for j in range(MXUS)]

    in_copy(0).wait()
    in_copy(2).start()
    for piece in pool_ops(0):
        done = piece()[1]
        if done:
            x_s[NTILE, done[0]:done[0] + SLAB, :] = done[1]
    for _, run, _ in project_ops(0):
        run({})
    xa_s[...] = x_s[:NA]

    rings = (ring0, ring1, ring2, ring3)
    rings16 = tuple(r.bitcast(BF16) for r in rings)
    RP, RY, RZ = T, T + T // 2, T + T // 2 + 48

    def round_a(i, _):
        zero = i >> 20
        nxt = jnp.minimum(i + 1, NKT - 1)

        @pl.when(i + 1 < NKT)
        def _():
            in_copy(i + 1).wait()

        @pl.when(i + 3 < NKT)
        def _():
            in_copy(i + 3).start()

        kk, vv = k_s[i], v_s[...]
        lanes = pl.ds(pl.multiple_of(i // 2 * T, T), T)
        for r in rings:
            r[RZ:RZ + T // 2, :T] = kk
            r[RZ:RZ + C // 2, T:2 * T] = vv
        for b in bufs:
            b[pl.ds(pl.multiple_of(at["K"] + i % 2 * (T // 2), 8), T // 2), lanes] = kk
        buf1[pl.ds(pl.multiple_of(VF0 + i % 2 * C, 8), C), lanes] = pltpu.bitcast(vf_s[...], I32)
        kk = kk[:, :C]

        def qk(q, j, pre):
            a = splice(lambda w0, w1: kk[w0 * 8:w1 * 8], T // SLAB, pre)
            s = jnp.dot(pltpu.bitcast(a, BF16), xa_s[4 * q + j], preferred_element_type=F32)
            put(rings[q % 4], 0, j, s)
            put(rings[q % 4], RY + 8, j, _max_over_vregs(s))
            return s

        def pv(q, j, pre):
            a = splice(lambda w0, w1: vv[w0 * 8:w1 * 8], C // SLAB, pre)
            d = jnp.dot(pltpu.bitcast(a, BF16), rings16[q % 4][2 * RP:2 * RP + T, j * T:(j + 1) * T],
                        preferred_element_type=F32)
            r0, c0 = state_pos(4 * q + j)
            put(buf1, r0, c0, get(buf1, r0, C, c0) * get(rings[q % 4], RY + 16, 1, j) + d)
            return d

        def softmax_ops(q):
            u = rings[q % 4]
            r0, c0 = state_pos(4 * q)
            st, pend = {}, {}

            def step(h):
                if h == 0:
                    m_old = get(buf1, r0 + C + 8, 8, c0, 4)
                    m = jnp.maximum(m_old, jnp.max(get(u, RY + 8, 8, 0, 4), axis=0, keepdims=True))
                    alpha = jnp.exp2(m_old - m)
                    put(buf1, r0 + C + 8, c0, m)
                    st.update(m=twice(m), l=get(buf1, r0 + C, 8, c0, 4) * alpha)
                    pend[2] = [functools.partial(put, u, RY + 16, 0, alpha)]
                elif h <= T // SLAB:
                    p = jnp.exp2(get(u, (h - 1) * SLAB, SLAB, 0, 4) - st["m"])
                    st["l"] = st["l"] + p[:8] + p[8:]
                    pend.setdefault(h + 1, []).append(
                        functools.partial(put16, rings16[q % 4], 2 * RP + (h - 1) * SLAB, 0, p.astype(BF16)))
                else:
                    put(buf1, r0 + C, c0, st["l"])
                for f in pend.pop(h, []):
                    f()
            return [functools.partial(step, h) for h in range(T // SLAB + 2)]

        nq, ahead, settle = NA // 4, 3, 9
        mats, qk_at, pv_at = [], {}, {}
        for q in range(nq + ahead):
            if q < nq:
                mats += [(T, functools.partial(qk, q, j), lambda p, w: rings[p][RZ + w * 8:RZ + w * 8 + 8, :C])
                         for j in range(4)]
                qk_at[q] = len(mats)
            if q == nq:
                project_at = len(mats)
                mats += project_ops(nxt)
            if q >= ahead:
                pv_at[q - ahead] = len(mats)
                mats += [(C, functools.partial(pv, q - ahead, j),
                          lambda p, w: rings[p][RZ + w * 8:RZ + w * 8 + 8, T:2 * T]) for j in range(4)]
        pool, held, done = pool_ops(nxt), [], {}

        def pool_step(u, jp, v):
            x_s[NTILE + 1 + zero, jp % 12 * 8:jp % 12 * 8 + 8, :] = v.astype(BF16)
            if held:
                acc, full = held.pop()
                put(u, RY + 24, jp % 4, acc)
                if full:
                    done[jp + settle] = full
            if jp in done:
                c, xs = done.pop(jp)
                x_s[NTILE, c:c + SLAB, :] = xs
            if jp < len(pool):
                held.append(pool[jp]())

        vecs, cycle, jp = [], 0, 0
        for q in range(nq):
            cycle = max(cycle, sum(m[0] for m in mats[:qk_at[q]]) // MXUS + MXU_LAT + 8)
            end = min(cycle + T + C, sum(m[0] for m in mats[:pv_at[q]]) // MXUS - 60)
            ops = softmax_ops(q)
            for h, f in enumerate(ops):
                before, run = pv_at[q], lambda v, f=f: f()
                if h % 2 == 1 and jp <= len(pool) + settle:
                    before = min(before, project_at)
                    run = lambda v, f=f, u=rings[q % 4], jp=jp: (pool_step(u, jp, v), f())
                    jp += 1
                vecs.append((cycle + (end - cycle) * h / len(ops), qk_at[q] - 1, before, rings[q % 4], q % 4, RY, run))
            cycle = end
        assert jp > len(pool) + settle
        emit(mats, vecs, zero)
        assert not held and not done
        return zero

    zero_a = jax.lax.fori_loop(0, NKT, round_a, 0)

    def handover_ops():
        def value(i, r0):
            return get(buf1, VF0 + i % 2 * C + r0, SLAB, i // 2)

        def mean(c):
            tot = functools.reduce(jnp.add, [value(i, c) for i in range(NKT)])
            vm_s[c:c + SLAB, :] = jnp.broadcast_to(
                jnp.sum(tot, axis=1, keepdims=True) * (1.0 / (NKT * T)), (SLAB, T))

        def finish(n):
            r0, c0 = state_pos(n)
            inv = pl.reciprocal(jnp.sum(get(buf1, r0 + C, 8, c0), axis=0, keepdims=True), full_range=False)
            o_s[n] = (get(buf1, r0, C, c0) * inv).astype(o_s.dtype)

        def a_sums(g, c, r0, r1):
            blocks = {(i, k): value(g * NK + k, i * CH + c) - vm_s[i * CH + c:i * CH + c + SLAB, :]
                      for i in range(NM) for k in range(NK) if SU[r0:r1, i, k].any()}
            a = jnp.concatenate([_lincomb(SU[r], lambda i, k: blocks[i, k]) for r in range(r0, r1)], axis=1)
            a = a.astype(BF16)
            if g == 0:
                for b16 in bufs16:
                    put16(b16, 2 * at["A"] + c, r0, a)
            put16(a16, g * CH + c, r0, a)
        return ([(10, functools.partial(mean, c)) for c in range(0, C, SLAB)]
                + [(22, functools.partial(finish, n)) for n in range(NA)]
                + [(20 if g else 50, functools.partial(a_sums, g, c, r, min(r + 8, R)))
                   for g in range(NG) for c in range(0, CH, SLAB) for r in range(0, R, 8)])

    def score_pos(g, s):
        a, b = divmod(g * NS + s, R // GW)
        return a * T, b * GW

    def qk_ops(row, par, zero):
        st, fresh = {}, []

        def copy(q, p, w):
            r0 = at["K"] + q % 2 * (T // 2) + w * 8
            return bufs[p][r0:r0 + 8, q // 2 * T:q // 2 * T + C]

        def qk(t, q, pre):
            if q == 0:
                st.clear()
            if q == 0 or (t * NKT + q) % MXUS == 0:
                st["x"] = x_s[NA + row * NT + t + zero * q]
            kk = splice(lambda w0, w1: k_s[q, w0 * 8:w1 * 8, :C], T // SLAB, pre)
            s = jnp.dot(pltpu.bitcast(kk, BF16), st["x"], preferred_element_type=F32)
            e = (q % NK, t)
            r0, c0 = score_pos(q // NK, WHEN[e])
            put(bufs[par], r0, c0 + GROUPS[WHEN[e]].index(e), s)
            fresh.append(_max_over_vregs(s))
            if q % 2 == 1 or q == NKT - 1:
                m = functools.reduce(jnp.maximum, ([st["m"]] if "m" in st else []) + fresh)
                w = [jnp.exp2(r - m) for r in fresh] + ([st["h"] * jnp.exp2(st["m"] - m)] if "m" in st else [])
                st.update(m=m, h=functools.reduce(jnp.add, w))
                fresh.clear()
            if q == NKT - 1:
                put(bufs[par], at["X"], t, jnp.concatenate([st["m"], st["h"]], axis=0))
            return s
        return [(T, functools.partial(qk, t, q), functools.partial(copy, q)) for t in range(NT) for q in range(NKT)]

    def softmax_ops(par):
        u = bufs[par]
        den, p, part, pend, saved = [None] * NT, {}, {}, {}, [0] * NT
        n, lag = NG * (T // SLAB) * NS, 2

        def row_max():
            m8 = get(u, at["X"], 8, 0, NT)
            m = jnp.broadcast_to(jnp.max(m8, axis=0, keepdims=True), (8, NT * T))
            put(u, at["H"], 0, get(u, at["X"] + 8, 8, 0, NT) * jnp.exp2(m8 - m))
            put(u, at["MAX"], 0, m)

        def balance():
            h = jnp.broadcast_to(jnp.sum(get(u, at["H"], 8, 0, NT), axis=0, keepdims=True), (8, NT * T))
            rho = jnp.concatenate([h[:, :T]] * (NT - 1), axis=1) * pl.reciprocal(h[:, T:], approx=True)
            put(u, at["RHO"], 1, rho)

        def flush(j):
            for f in pend.pop(j, []):
                f()

        def step(j):
            i, s = divmod(j, NS)
            g, h = divmod(i, T // SLAB)
            r0, c0 = score_pos(g, s)
            m = twice(jnp.concatenate([get(u, at["MAX"], 8, t) for _, t in GROUPS[s]], axis=1))
            e = jnp.exp2(get(u, r0 + h * SLAB, SLAB, c0, GW) - m)
            for w, (k, t) in enumerate(GROUPS[s]):
                p[k, t] = e[:, w * T:(w + 1) * T]
                if t > 0:
                    p[k, t] = p[k, t] * twice(get(u, at["RHO"], 8, t))
            for x, a, b, sign in TEMPS:
                if WHEN[x] == s:
                    p[x] = p[a] + p[b] if sign > 0 else p[a] - p[b]
            for t in range(NT):
                uses = [WHEN[x] for x in SUMS[t]]
                for x in SUMS[t]:
                    if WHEN[x] == s:
                        den[t] = p[x][:8] + p[x][8:] if den[t] is None else den[t] + p[x][:8] + p[x][8:]
                if s in uses and min([q for q in uses if q > s] + [uses[0] + NS]) - s > 2 and j + 3 < n:
                    pend.setdefault(j + 3, []).append(
                        functools.partial(put, u, at["L"] + saved[t] % (NG * 8) * 8, t, den[t]))
                    saved[t] += 1
            for r in range(R):
                for when, x, sign in PROG[r]:
                    if when == s:
                        part[r] = p[x] if r not in part else part[r] + p[x] if sign > 0 else part[r] - p[x]
            ready = [r for r in range(R) if PROG[r][-1][0] == s]
            b = jnp.concatenate([part.pop(r) for r in ready], axis=1).astype(BF16)
            pend.setdefault(j + lag, []).append(
                functools.partial(put16, bufs16[par], 2 * at["B"] + g * T + h * SLAB, ready[0], b))
            flush(j)

        def invert():
            assert not pend
            tot = jnp.sum(jnp.concatenate(den, axis=1), axis=0, keepdims=True)
            put(u, at["INV"], 0, pl.reciprocal(jnp.broadcast_to(tot, (8, NT * T)), full_range=False))
        return ([[row_max], [], [], [], [balance], [], []],
                [[functools.partial(step, j)] for j in range(n)],
                [[functools.partial(flush, j)] for j in range(n, n + lag)] + [[invert]])

    def pv_ops(par):
        acc = {}

        def copy(r, p, w):
            return bufs16[p][2 * at["A"] + w * SLAB:2 * at["A"] + (w + 1) * SLAB, r * T:(r + 1) * T]

        def pv(r, g, pre):
            a = splice(lambda w0, w1: a16[g * CH + w0 * SLAB:g * CH + w1 * SLAB, r * T:(r + 1) * T], CH // SLAB, pre)
            b = bufs16[par][2 * at["B"] + g * T:2 * at["B"] + (g + 1) * T, r * T:(r + 1) * T]
            d = jnp.dot(a, b, preferred_element_type=F32)
            acc[r] = d if g == 0 else d + acc[r]
            if g == NG - 1:
                put(bufs[par], at["M"], r, acc[r])
            return acc[r]
        return [(CH, functools.partial(pv, r, g), functools.partial(copy, r) if g == 0 else None)
                for r in range(R) for g in range(NG)]

    def output_ops(row, par):
        u = bufs[par]
        both = (SW[:, 0] == SW[:, 1]) * SW[:, 0]
        base = jnp.where(row < 0, NTILE, NA + row * NT)

        def shared(t, c):
            return functools.partial(put, u, at["F"], 0, _lincomb(both[:, t], lambda q: get(u, at["M"] + c, SLAB, q)))

        def finish(i, t, c):
            o = _lincomb(np.append(SW[:, i, t] - both[:, t], 1),
                         lambda q: get(u, at["M"] + c, SLAB, q) if q < R else get(u, at["F"], SLAB, 0))
            rows = slice(i * CH + c, i * CH + c + SLAB)
            o = (o * twice(get(u, at["INV"], 8, t)) + vm_s[rows, :]).astype(o_s.dtype)
            o_s[base + t, rows, :] = o
            return functools.partial(put16, bufs16[par], 2 * at["OUT"], 0, o)
        return [f for c in range(0, CH, SLAB) for t in range(NT) for f in (
            functools.partial(shared, t, c), functools.partial(finish, 0, t, c), functools.partial(finish, 1, t, c))]

    adds = [sum(WHEN[x[0]] == s for x in TEMPS) + sum(w == s for pr in PROG for w, _, _ in pr[1:]) for s in range(NS)]
    outs = [sum(pr[-1][0] == s for pr in PROG) for s in range(NS)]

    def run_steps(steps, zero, extra=()):
        order, count = [], [0, 0]
        for s, (row1, _, on3, _, par) in enumerate(steps):
            for kind, ops in enumerate((qk_ops(row1, par, zero) if row1 is not None else [],
                                        pv_ops(par) if on3 else [])):
                for i, op in enumerate(ops):
                    order.append((round(s + (i - count[kind] % MXUS) / len(ops), 6), kind, s, op))
                    count[kind] += 1
        order.sort(key=lambda e: e[:2])
        issue = np.cumsum([0] + [e[3][0] / MXUS for e in order])
        real = np.concatenate([[0], issue + MXU_LAT - 70, [issue[-1] + 1000]])
        pace = np.cumsum([0, MXU_LAT - 70] + [e[3][0] / MXUS * (1.1 if e[1] else 1) for e in order] + [1000])
        vecs, start = [], 0
        for s, (_, on2, _, row4, par) in enumerate(steps):
            span = sum(e[3][0] for e in order if e[2] == s) / MXUS
            after = max([n for n, e in enumerate(order) if e[2] < s], default=-1)
            before = min([n for n, e in enumerate(order) if e[2] > s], default=len(order))
            head, body, tail = softmax_ops(1 - par) if on2 else ([], [], [])
            last = output_ops(row4, 1 - par) if row4 is not None else []
            if on2:
                slots = [j for j in range(len(body)) if j % NS < 3]
                assert len(slots) >= len(last)
                for i, f in enumerate(last):
                    j, box = slots[i * len(slots) // len(last)], []
                    body[j].append(lambda f=f, box=box: box.append(f()))
                    body[j + 1].append(lambda box=box: box.pop()())
                cost = [24 + 0.5 * adds[(j - 1) % NS] + outs[(j - 2) % NS] + 3 * max(len(fs) - 1, 0)
                        for j, fs in enumerate(head + body + tail, -len(head))]
            else:
                timed = [(1, lambda f=f: f()()) for f in last] + list(extra if s == 0 else ())
                cost, body = [c for c, _ in timed], [[f] for _, f in timed]
            first = 40 if s == 0 else issue[min(after // MXUS * MXUS + MXUS, len(order))] + MXU_LAT + 10
            user = [n for n, e in enumerate(order) if e[2] > s and e[1] == 1]
            final = issue[user[0] // MXUS * MXUS] - 160 if user else start + span + 100
            if before < len(order):
                final = min(final, issue[before // MXUS * MXUS] + MXU_LAT - 10)
            lo, hi = np.interp([first, final], real, pace)
            for fs, pos in zip(head + body + tail, np.cumsum([0] + cost) / max(sum(cost), 1)):
                vecs.append((float(np.interp(lo + (hi - lo) * pos, pace, real)) if span else 0, after, before,
                             bufs[1 - par], 1 - par, at["PACE"], lambda v, fs=fs: [f() for f in fs]))
            start += span
        emit([e[3] for e in order], vecs, zero)

    rows = (NTILE - NA) // NT
    iters = (rows - 2) // UNROLL
    block = NT * UNROLL
    lead = (NA - NT) // block - 1
    assert NA + rows * NT == NTILE and 2 + iters * UNROLL == rows and H % block == 0 and lead > 0
    run_steps([(0, False, False, None, 0), (1, True, False, None, 1)], zero_a, handover_ops())

    def main(i, _):
        out_copy((lead + i) * block, block).start()
        run_steps([(i * UNROLL + s + 2, True, True, i * UNROLL + s - 1, s % 2) for s in range(UNROLL)], i >> 20)

    jax.lax.fori_loop(0, iters, main, None)
    sent, rest = (lead + iters) * block, NTILE - 3 * NT
    out_copy(sent, rest - sent).start()
    out_copy(0, lead * block).start()
    run_steps([(None, r + 1 < rows, r < rows, r - 1, r % 2) for r in range(rows - 2, rows + 1)], zero_a)
    out_copy(rest, NTILE - rest).start()
    pltpu.make_async_copy(o_hbm, o_hbm, out_sem).wait()


@jax.jit
def pallas_standalone__window_attn_twins__vision_kernel(
    x: jax.Array,
    wq: jax.Array,
    wkv: jax.Array,
    wo: jax.Array,
):
    B, H, W, C = x.shape
    ntile = H * W // T
    nkt = ntile // (WIN * WIN)
    assert B == 1 and W % T == 0 and H % (WIN * WIN) == 0 and nkt % NK == 0 and C % (NM * SLAB) == 0 and C <= T
    out = pl.pallas_call(
        _kernel,
        in_specs=[pl.BlockSpec(memory_space=pl.ANY)] * 4,
        out_specs=pl.BlockSpec(memory_space=pl.ANY),
        out_shape=jax.ShapeDtypeStruct((H, C, W), x.dtype),
        scratch_shapes=[
            pltpu.VMEM((ntile + 2, C, T), x.dtype),
            pltpu.VMEM((ntile + NT, C, T), x.dtype),
            pltpu.VMEM((NA, C, T), x.dtype),
            pltpu.VMEM(wq.shape, wq.dtype),
            pltpu.VMEM(wkv.shape, wkv.dtype),
            pltpu.VMEM(wo.shape, wo.dtype),
            pltpu.VMEM((2 * C, C), BF16),
            pltpu.VMEM((nkt, T // 2, T), I32),
            pltpu.VMEM((C // 2, T), I32),
            pltpu.VMEM((C, T), F32),
            pltpu.VMEM((nkt // NK * C // NM // 2, R * T), I32),
            pltpu.VMEM((C, T), F32),
            *[pltpu.VMEM((2 * T + 48, 4 * T), I32)] * 4,
            *[pltpu.VMEM((_layout(C, nkt)["END"], R * T), I32)] * 2,
            pltpu.SemaphoreType.DMA((nkt,)),
            pltpu.SemaphoreType.DMA((3,)),
            pltpu.SemaphoreType.DMA(()),
        ],
        compiler_params=pltpu.CompilerParams(vmem_limit_bytes=120 << 20),
    )(jnp.transpose(x, (0, 1, 3, 2)).reshape(H, C, W), wq, wkv, wo)
    return jnp.transpose(out.reshape(B, H, C, W), (0, 1, 3, 2))
```
